```python
import jax
import jax.numpy as jnp

def _softmax(x, axis=-1):
    return jax.nn.softmax(x, axis=axis)

def _gelu(x):
    return jax.nn.gelu(x, approximate=True)

def _silu(x):
    return jax.nn.silu(x)

def _sigmoid(x):
    return jax.nn.sigmoid(x)

def _layernorm(x, axis=-1, eps=1e-05):
    m = jnp.mean(x, axis=axis, keepdims=True)
    v = jnp.var(x, axis=axis, keepdims=True)
    return (x - m) / jnp.sqrt(v + eps)

def _scatter_add(tgt, idx, src, axis=0):
    return tgt.at[idx].add(src)

def _segment_sum(src, seg, n):
    return jax.ops.segment_sum(src, seg, n)

class _Rng:

    def __init__(self, key):
        self._k = key

    def _next(self):
        self._k, sub = jax.random.split(self._k)
        return sub

    def normal(self, shape):
        return jax.random.normal(self._next(), shape, dtype=jnp.bfloat16)

    def randint(self, lo, hi, shape):
        return jax.random.randint(self._next(), shape, lo, hi, dtype=jnp.int32)

    def uniform(self, shape, lo=0.0, hi=1.0):
        return jax.random.uniform(self._next(), shape, jnp.bfloat16, lo, hi)

    def permutation(self, n):
        return jax.random.permutation(self._next(), n)
kernel_name = 'concat_heads__softmax_full_mha__memory_aug_recurrent_mem_tr__prompt'

def setup_inputs():
    _rng = _Rng(jax.random.key(int.from_bytes(__import__("os").urandom(4), "little")))
    _w = lambda a: (lambda t: t.astype(jnp.bfloat16) if jnp.issubdtype(t.dtype, jnp.floating) else t)(jnp.asarray(a))

    def _A_setup():
        B, S, D = (1, 2048, 1024)
        return {'x': _w((lambda *s: _rng.normal(s) * 0.05)(B, S, D)), 'wqkv': _w((lambda *s: _rng.normal(s) * 0.05)(D, 3 * D)), 'wo': _w((lambda *s: _rng.normal(s) * 0.05)(D, D))}
    _A_in = _A_setup()

    def _B_setup():
        B, S, Dm = (1, 2048, 1024)
        H, Dh = (32, 128)
        M, seg = (8, 32)
        seg = min(seg, S)
        S = S // seg * seg
        return {'x': _w((lambda *s: _rng.normal(s) * 0.05)(B, S, Dm)), 'mem0': _w((lambda *s: _rng.normal(s) * 0.05)(B, M, Dm)), 'Wq': _w((lambda *s: _rng.normal(s) * 0.05)(Dm, H, Dh) * Dm ** (-0.5)), 'Wk': _w((lambda *s: _rng.normal(s) * 0.05)(Dm, H, Dh) * Dm ** (-0.5)), 'Wv': _w((lambda *s: _rng.normal(s) * 0.05)(Dm, H, Dh) * Dm ** (-0.5)), 'Wo': _w((lambda *s: _rng.normal(s) * 0.05)(H, Dh, Dm) * (H * Dh) ** (-0.5)), 'seg_len': seg}
    _B_in = _B_setup()
    return {'A_x': _A_in['x'], 'A_wqkv': _A_in['wqkv'], 'A_wo': _A_in['wo'], 'B_x': _B_in['x'], 'B_mem0': _B_in['mem0'], 'B_Wq': _B_in['Wq'], 'B_Wk': _B_in['Wk'], 'B_Wv': _B_in['Wv'], 'B_Wo': _B_in['Wo'], 'B_seg_len': _B_in['seg_len']}

def reference(A_x, A_wqkv, A_wo, B_x, B_mem0, B_Wq, B_Wk, B_Wv, B_Wo, B_seg_len):

    def _A_ref(x, wqkv, wo):
        B, S, D = x.shape
        H = 32
        Dh = D // H
        qkv = (lambda x, *d: x.transpose(*d))((x @ wqkv).reshape(B, S, 3, H, Dh), 2, 0, 3, 1, 4)
        q, k, v = (qkv[0], qkv[1], qkv[2])
        scale = Dh ** (-0.5)
        scores = jnp.einsum('bhqd,bhkd->bhqk', q, k) * scale
        p = _softmax(scores, axis=-1)
        o = jnp.einsum('bhqk,bhkd->bhqd', p, v)
        return (lambda x, *d: x.transpose(*d))(o, 0, 2, 1, 3).reshape(B, S, D) @ wo

    def _B_ref(x, mem0, Wq, Wk, Wv, Wo, seg_len):
        B, S, Dm = x.shape
        H, Dh = (Wq.shape[1], Wq.shape[2])
        M = mem0.shape[1]
        scale = Dh ** (-0.5)
        n_seg = S // seg_len
        L = M + seg_len
        idx = jnp.arange(L)
        mask = (idx[:, None] < M) | (idx[:, None] >= idx[None, :])
        mem = mem0
        outs = []
        for s in range(n_seg):
            xs = x[:, s * seg_len:(s + 1) * seg_len, :].copy()
            h = jnp.concatenate([mem, xs], axis=1)
            q = jnp.einsum('btd,dhe->bhte', h, Wq)
            k = jnp.einsum('btd,dhe->bhte', h, Wk)
            v = jnp.einsum('btd,dhe->bhte', h, Wv)
            scores = jnp.einsum('bhqe,bhke->bhqk', q, k) * scale
            scores = jnp.where(mask[None, None], scores, -1000000000.0)
            p = _softmax(scores, axis=-1)
            o = jnp.einsum('bhqk,bhke->bhqe', p, v)
            o = jnp.einsum('bhte,hed->btd', o, Wo)
            mem = o[:, :M, :].copy()
            outs.append(o[:, M:, :])
        return jnp.concatenate(outs, axis=1)
    a = _A_ref(A_x, A_wqkv, A_wo)
    b = _B_ref(B_x, B_mem0, B_Wq, B_Wk, B_Wv, B_Wo, B_seg_len)
    return jnp.concatenate([a, b], axis=-1)
```

```python
import functools

import jax
import jax.numpy as jnp
from jax import lax
from jax.experimental import pallas as pl
from jax.experimental.pallas import tpu as pltpu

_LOG2E = 1.4426950408889634
_NN = (((1,), (0,)), ((), ()))
_NT = (((1,), (1,)), ((), ()))
_TN = (((0,), (0,)), ((), ()))
_BF = jnp.bfloat16
_F32 = jnp.float32
_U32 = jnp.uint32


def _dot(a, b, dims=_NN):
    return lax.dot_general(a, b, dims, preferred_element_type=_F32)


def _as_bf16(u):
    return pltpu.bitcast(u, _BF)


def _as_u32(b):
    return pltpu.bitcast(b, _U32)


def _round_bf16(x):
    return x.astype(_BF).astype(_F32)


def _recip(l):
    r0 = pltpu.reciprocal(l, approx=True)
    return r0 * (2.0 - l * r0)


S = 2048
D = 1024
HA, DHA = 32, 32
HB, DHB = 32, 128
MEM = 8
SEG = 32
LB = MEM + SEG

MB1 = 256
QT = 512
KB = 128
NUNITS = HA * (S // QT)
GB = 8
DCH = 16


def _kernel(xa_hbm, wqkv_hbm, woa_hbm, xb_hbm, mem_ref, wq_hbm, wk_hbm, wv_hbm, wob_hbm,
            out_hbm,
            wqkv_v, xa_v, qT, kA, vT, s0, s1, oT, woa_v,
            stage, wB, wob_v, xb_v, o_scr, outb_v,
            sems):
    SEM_XA, SEM_WQKV, SEM_MISC, SEM_STAGE, SEM_OUTA, SEM_OUTB = 0, 8, 11, 14, 20, 21
    n_mb = S // MB1

    def xa_copy(i):
        return pltpu.make_async_copy(xa_hbm.at[pl.ds(i * MB1, MB1)], xa_v.at[pl.ds(i * MB1, MB1)],
                                     sems.at[SEM_XA + i])

    def wqkv_copy(j):
        return pltpu.make_async_copy(wqkv_hbm.at[:, pl.ds(j * D, D)], wqkv_v.at[:, pl.ds(j * D, D)],
                                     sems.at[SEM_WQKV + j])

    woa_copy = pltpu.make_async_copy(woa_hbm, woa_v, sems.at[SEM_MISC])
    xb_copy = pltpu.make_async_copy(xb_hbm, xb_v, sems.at[SEM_MISC + 1])
    wob_copy = pltpu.make_async_copy(wob_hbm, wob_v, sems.at[SEM_MISC + 2])
    wsrc = (wq_hbm, wk_hbm, wv_hbm)

    def stage_copy(c, slot, j):
        return pltpu.make_async_copy(wsrc[j].at[pl.ds(c * DCH, DCH)], stage.at[slot * 3 + j],
                                     sems.at[SEM_STAGE + slot * 3 + j])

    xa_copy(0).start()
    for j in range(3):
        wqkv_copy(j).start()
    for i in range(1, n_mb):
        xa_copy(i).start()
    for j in range(3):
        stage_copy(0, 0, j).start()
    woa_copy.start()
    xb_copy.start()
    wob_copy.start()

    qscale = float(DHA) ** -0.5 * _LOG2E
    for j in range(3):
        wqkv_copy(j).wait()

    def p1_body(i, _):
        pltpu.make_async_copy(xa_hbm.at[pl.ds(0, MB1)], xa_v.at[pl.ds(0, MB1)],
                              sems.at[SEM_XA + i]).wait()
        r0 = pl.multiple_of(i * MB1, MB1)
        x = xa_v[pl.ds(r0, MB1), :]
        q = _dot(x, wqkv_v[:, 0:D]) * qscale
        qT[:, pl.ds(r0, MB1)] = _as_u32(q.astype(_BF).T)
        k = _dot(x, wqkv_v[:, D:2 * D])
        kA[pl.ds(pl.multiple_of(i * (MB1 // 2), MB1 // 2), MB1 // 2), :] = _as_u32(k.astype(_BF))
        v = _dot(x, wqkv_v[:, 2 * D:3 * D])
        vT[:, pl.ds(r0, MB1)] = _as_u32(v.astype(_BF).T)
        return 0

    lax.fori_loop(0, n_mb, p1_body, 0)

    NKB = S // KB
    rowg = lax.broadcasted_iota(jnp.int32, (64, QT), 0) // 16

    def load_qm(u):
        qt = u >> 5
        h = u & (HA - 1)
        g = h >> 2
        qg = qT[pl.ds(pl.multiple_of(g * 64, 64), 64), pl.ds(pl.multiple_of(qt * QT, QT), QT)]
        return _as_bf16(jnp.where(rowg == (h & 3), qg, jnp.uint32(0)))

    def pass1_blk(u, qm, kb, s_ref, m8):
        g = (u & (HA - 1)) >> 2
        kk = _as_bf16(kA[pl.ds(kb * (KB // 2), KB // 2), pl.ds(pl.multiple_of(g * 128, 128), 128)])
        s = _dot(kk, qm)
        s_ref[pl.ds(kb * KB, KB), :] = s
        mm = jnp.max(s.reshape(KB // 8, 8, QT), axis=0)
        return mm if m8 is None else jnp.maximum(m8, mm)

    def pass2_blk(u, m, kb, s_ref, l8, acc):
        h = u & (HA - 1)
        p = jnp.exp2(s_ref[pl.ds(kb * KB, KB), :] - m)
        ls = jnp.sum(p.reshape(KB // 8, 8, QT), axis=0)
        l8 = ls if l8 is None else l8 + ls
        vt = _as_bf16(vT[pl.ds(pl.multiple_of(h * 16, 16), 16), pl.ds(kb * KB, KB)])
        pv = _dot(vt, p.astype(_BF))
        acc = pv if acc is None else acc + pv
        return l8, acc

    def finish(u, l8, acc):
        qt = u >> 5
        h = u & (HA - 1)
        r = _recip(jnp.sum(l8, axis=0, keepdims=True))
        oT[pl.ds(pl.multiple_of(h * 16, 16), 16), pl.ds(pl.multiple_of(qt * QT, QT), QT)] = (
            _as_u32((acc * r).astype(_BF)))

    def pass1_all(u, s_ref):
        qm = load_qm(u)
        m8 = None
        for kb in range(NKB):
            m8 = pass1_blk(u, qm, kb, s_ref, m8)
        return jnp.max(m8, axis=0, keepdims=True)

    def unit(u, m, s_ref, do_pass1):
        if do_pass1:
            qm = load_qm(u + 2)
        m8 = None
        l8 = acc = None
        for kb in range(NKB):
            l8, acc = pass2_blk(u, m, kb, s_ref, l8, acc)
            if do_pass1:
                m8 = pass1_blk(u + 2, qm, kb, s_ref, m8)
        finish(u, l8, acc)
        return jnp.max(m8, axis=0, keepdims=True) if do_pass1 else None

    j_iota = lax.broadcasted_iota(jnp.int32, (8, 128), 0)

    def relayout_chunk(c, slot):
        for j in range(3):
            V = [_as_u32(stage[slot * 3 + j, d]) for d in range(DCH)]
            for g2 in range(2):
                Vg = [v[g2 * 8:(g2 + 1) * 8] for v in V]
                Ls, Hs = [], []
                for i in range(8):
                    a, b = Vg[2 * i], Vg[2 * i + 1]
                    Ls.append((a & jnp.uint32(0xFFFF)) | (b << 16))
                    Hs.append((a >> 16) | (b & jnp.uint32(0xFFFF0000)))
                for bsel, X in ((0, Ls), (1, Hs)):
                    X = list(X)
                    for s in (4, 2, 1):
                        mask = (j_iota & s) == 0
                        for i in range(8):
                            if i & s:
                                continue
                            x, y = X[i], X[i + s]
                            X[i] = jnp.where(mask, x, pltpu.roll(y, s, 0))
                            X[i + s] = jnp.where(mask, pltpu.roll(x, 8 - s, 0), y)
                    for jj in range(8):
                        wB[j * HB + g2 * 16 + 2 * jj + bsel, pl.ds(pl.multiple_of(c * 8, 8), 8), :] = X[jj]

    m_a = pass1_all(0, s0)
    m_b = pass1_all(1, s1)
    n_it = NUNITS // 2
    assert n_it == D // DCH

    def p2_body(i, carry, last):
        ma, mb = carry
        slot = i & 1
        if not last:
            for j in range(3):
                stage_copy(i + 1, 1 - slot, j).start()
        for j in range(3):
            stage_copy(i, slot, j).wait()
        relayout_chunk(i, slot)
        ma = unit(2 * i, ma, s0, not last)
        mb = unit(2 * i + 1, mb, s1, not last)
        return (ma, mb)

    carry = lax.fori_loop(0, n_it - 1, functools.partial(p2_body, last=False), (m_a, m_b))
    p2_body(n_it - 1, carry, True)

    woa_copy.wait()

    def outa_copy(i):
        r0 = pl.multiple_of(i * MB1, MB1)
        return pltpu.make_async_copy(xa_v.at[pl.ds(r0, MB1)], out_hbm.at[pl.ds(r0, MB1), pl.ds(0, D)],
                                     sems.at[SEM_OUTA])

    def p3_body(i, _):
        r0 = pl.multiple_of(i * MB1, MB1)
        o = _dot(_as_bf16(oT[:, pl.ds(r0, MB1)]), woa_v[...], _TN)
        xa_v[pl.ds(r0, MB1), :] = o.astype(_BF)
        outa_copy(i).start()
        return 0

    lax.fori_loop(0, n_mb, p3_body, 0)

    xb_copy.wait()
    wob_copy.wait()
    ri = lax.broadcasted_iota(jnp.int32, (LB, LB), 0)
    ci = lax.broadcasted_iota(jnp.int32, (LB, LB), 1)
    bmask = (ri < MEM) | (ri >= ci)
    bscale = float(DHB) ** -0.5 * _LOG2E
    NG = HB // GB

    def b_attn_head(q, k, v):
        s = _dot(q, k, _NT)
        s = jnp.where(bmask, s, -1e9)
        mx = jnp.max(s, axis=1, keepdims=True)
        p = jnp.exp2((s - mx) * bscale)
        l = jnp.sum(p, axis=1, keepdims=True)
        o = _dot(p, v)
        return _round_bf16(o * _recip(l))

    def outb_copy(s_):
        r0 = pl.multiple_of(s_ * SEG, SEG)
        return pltpu.make_async_copy(outb_v.at[pl.ds(r0, SEG)], out_hbm.at[pl.ds(r0, SEG), pl.ds(D, D)],
                                     sems.at[SEM_OUTB])

    def b_step(s_, mem):
        r0 = pl.multiple_of(s_ * SEG, SEG)
        h = jnp.concatenate([mem, xb_v[pl.ds(r0, SEG), :].astype(_F32)], axis=0)

        def qkv(g):
            def proj(j):
                w = jnp.concatenate([_as_bf16(wB[j * HB + g * GB + t]) for t in range(GB)], axis=1)
                return _dot(h, w)
            return proj(0), proj(1).astype(_BF), proj(2).astype(_BF)

        def attn(g, q, k, v):
            for t in range(GB):
                c0 = (g * GB + t) * DHB
                sl = slice(t * DHB, (t + 1) * DHB)
                o_scr[:, c0:c0 + DHB] = b_attn_head(q[:, sl], k[:, sl], v[:, sl])

        cur = qkv(0)
        for g in range(NG):
            nxt = qkv(g + 1) if g + 1 < NG else None
            attn(g, *cur)
            cur = nxt
        acc = _dot(o_scr[...], wob_v[...])
        outb_v[pl.ds(r0, SEG), :] = acc[MEM:, :].astype(_BF)
        outb_copy(s_).start()
        return _round_bf16(acc[:MEM, :])

    lax.fori_loop(0, S // SEG, b_step, mem_ref[...].astype(_F32))

    pltpu.make_async_copy(xa_v, out_hbm.at[:, pl.ds(0, D)], sems.at[SEM_OUTA]).wait()
    pltpu.make_async_copy(outb_v, out_hbm.at[:, pl.ds(D, D)], sems.at[SEM_OUTB]).wait()


@functools.partial(jax.jit, static_argnames=("B_seg_len",))
def pallas_concat_heads__softmax_full_mha__memory_aug_recurrent_mem_tr__prompt_kernel(
    A_x, A_wqkv, A_wo, B_x, B_mem0, B_Wq, B_Wk, B_Wv, B_Wo, B_seg_len,
):
    assert A_x.shape == (1, S, D) and A_wqkv.shape == (D, 3 * D) and A_wo.shape == (D, D)
    assert B_x.shape == (1, S, D) and B_mem0.shape == (1, MEM, D)
    assert B_Wq.shape == B_Wk.shape == B_Wv.shape == (D, HB, DHB) and B_Wo.shape == (HB, DHB, D)
    assert int(B_seg_len) == SEG

    any_spec = pl.BlockSpec(memory_space=pl.ANY)
    vmem_spec = pl.BlockSpec(memory_space=pltpu.VMEM)
    scratch = [
        pltpu.VMEM((D, 3 * D), _BF),
        pltpu.VMEM((S, D), _BF),
        pltpu.VMEM((D // 2, S), _U32),
        pltpu.VMEM((S // 2, D), _U32),
        pltpu.VMEM((D // 2, S), _U32),
        pltpu.VMEM((S, QT), _F32),
        pltpu.VMEM((S, QT), _F32),
        pltpu.VMEM((D // 2, S), _U32),
        pltpu.VMEM((D, D), _BF),
        pltpu.VMEM((6, DCH, HB, DHB), _BF),
        pltpu.VMEM((3 * HB, D // 2, DHB), _U32),
        pltpu.VMEM((HB * DHB, D), _BF),
        pltpu.VMEM((S, D), _BF),
        pltpu.VMEM((LB, HB * DHB), _F32),
        pltpu.VMEM((S, D), _BF),
        pltpu.SemaphoreType.DMA((22,)),
    ]
    out = pl.pallas_call(
        _kernel,
        out_shape=jax.ShapeDtypeStruct((S, 2 * D), _BF),
        in_specs=[any_spec, any_spec, any_spec, any_spec, vmem_spec, any_spec, any_spec, any_spec, any_spec],
        out_specs=any_spec,
        scratch_shapes=scratch,
        compiler_params=pltpu.CompilerParams(vmem_limit_bytes=110 * 1024 * 1024),
        name="concat_mha_rmt",
    )(A_x.reshape(S, D), A_wqkv, A_wo, B_x.reshape(S, D), B_mem0.reshape(MEM, D),
      B_Wq, B_Wk, B_Wv, B_Wo.reshape(HB * DHB, D))
    return out.reshape(1, S, 2 * D)
```

```python
import functools

import jax
import jax.numpy as jnp
from jax import lax
from jax.experimental import pallas as pl
from jax.experimental.pallas import tpu as pltpu

_LOG2E = 1.4426950408889634
_NN = (((1,), (0,)), ((), ()))
_NT = (((1,), (1,)), ((), ()))
_TN = (((0,), (0,)), ((), ()))
_BF = jnp.bfloat16
_F32 = jnp.float32
_U32 = jnp.uint32


def _dot(a, b, dims=_NN):
    return lax.dot_general(a, b, dims, preferred_element_type=_F32)


def _as_bf16(u):
    return pltpu.bitcast(u, _BF)


def _as_u32(b):
    return pltpu.bitcast(b, _U32)


def _round_bf16(x):
    return x.astype(_BF).astype(_F32)


def _recip(l):
    r0 = pltpu.reciprocal(l, approx=True)
    return r0 * (2.0 - l * r0)


S = 2048
D = 1024
HA, DHA = 32, 32
HB, DHB = 32, 128
MEM = 8
SEG = 32
LB = MEM + SEG

MB1 = 256
PIECE = 128
MB3 = 512
QT = 512
KB = 128
NKB = S // KB
NUNITS = HA * (S // QT)
GB = 2
TICKS = (1, 2, 0, 1, 4)
DCH = 16
NGRP = S // MB1
GCH = D // DCH // NGRP
DG = DCH * GCH
OCH = HB * DHB // (D // DCH)
OG = OCH * GCH
NSLOT = 3

SEM_XA = 0
SEM_WQKV = SEM_XA + S // MB1
SEM_MISC = SEM_WQKV + 3
SEM_STAGE = SEM_MISC + 3
SEM_OUT = SEM_STAGE + 4 * NSLOT
NSEM = SEM_OUT + 2


def _kernel(xa_hbm, wqkv_hbm, woa_hbm, xb_hbm, mem_hbm, wq_hbm, wk_hbm, wv_hbm, wob_hbm,
            out_hbm,
            wqkv_v, xa_v, qT, kA, vT, s0, s1, oT, woa_v,
            stage, stage_o, wB, wob_v, xb_v, mem_v, o_scr, outb_v, zsm,
            sems):
    n_mb = S // MB1
    sem_xa = lambda i: sems.at[SEM_XA + i]
    sem_wqkv = lambda j: sems.at[SEM_WQKV + j]
    sem_misc = lambda j: sems.at[SEM_MISC + j]
    sem_stage = lambda j: sems.at[SEM_STAGE + j]
    sem_out = lambda j: sems.at[SEM_OUT + j]
    zsm[0] = 0

    def xa_copy(i):
        return pltpu.make_async_copy(xa_hbm.at[pl.ds(i * MB1, MB1)], xa_v.at[pl.ds(i * MB1, MB1)],
                                     sem_xa(i))

    def wqkv_copy(j):
        return pltpu.make_async_copy(wqkv_hbm.at[:, pl.ds(j * D, D)], wqkv_v.at[:, pl.ds(j * D, D)],
                                     sem_wqkv(j))

    woa_copy = pltpu.make_async_copy(woa_hbm, woa_v, sem_misc(0))
    xb_copy = pltpu.make_async_copy(xb_hbm, xb_v, sem_misc(1))
    mem_copy = pltpu.make_async_copy(mem_hbm, mem_v, sem_misc(2))
    wsrc = (wq_hbm, wk_hbm, wv_hbm)

    def stage_copy(g, slot, j):
        sem = sem_stage(slot * 4 + j)
        if j == 3:
            return pltpu.make_async_copy(wob_hbm.at[pl.ds(g * OG, OG)], stage_o.at[slot], sem)
        return pltpu.make_async_copy(wsrc[j].at[pl.ds(g * DG, DG)], stage.at[slot * 3 + j], sem)

    def group_start(g, slot):
        for j in range(4):
            stage_copy(g, slot, j).start()

    def group_wait(g, slot):
        for j in range(4):
            stage_copy(g, slot, j).wait()

    P1_ORDER = (0, 2, 1)
    xa_copy(0).start()
    for j in P1_ORDER:
        wqkv_copy(j).start()
    xa_copy(1).start()
    group_start(0, 0)
    xa_copy(2).start()
    group_start(1, 1)
    xa_copy(3).start()
    group_start(2, 2)
    for i in range(4, n_mb):
        xa_copy(i).start()
    mem_copy.start()

    j_iota = lax.broadcasted_iota(jnp.int32, (8, 128), 0)

    def relayout_tasks(g, slot, c):
        row = pl.multiple_of(g * (DG // 2) + c * 8, 8)
        tasks = []
        for j in range(3):
            for g2 in range(2):
                for odd in range(2):
                    def task(j=j, g2=g2, odd=odd):
                        X = []
                        for i in range(8):
                            a = _as_u32(stage[slot * 3 + j, c * DCH + 2 * i, g2 * 16:(g2 + 1) * 16, :])
                            b = _as_u32(stage[slot * 3 + j, c * DCH + 2 * i + 1, g2 * 16:(g2 + 1) * 16, :])
                            if odd == 0:
                                X.append((a & jnp.uint32(0xFFFF)) | (b << 16))
                            else:
                                X.append((a >> 16) | (b & jnp.uint32(0xFFFF0000)))
                        for s in (4, 2, 1):
                            mask = (j_iota & s) == 0
                            for i in range(8):
                                if i & s:
                                    continue
                                x, y = X[i], X[i + s]
                                X[i] = jnp.where(mask, x, pltpu.roll(y, s, 0))
                                X[i + s] = jnp.where(mask, pltpu.roll(x, 8 - s, 0), y)
                        for jj in range(8):
                            wB[j * HB + g2 * 16 + 2 * jj + odd, pl.ds(row, 8), :] = X[jj]
                        return wB[zsm[0], pl.ds(row, 8), :]
                    tasks.append(task)
        orow = pl.multiple_of(g * (OG // 2) + c * (OCH // 2), OCH // 2)
        for q in range(4):
            def task(q=q):
                wob_v[pl.ds(orow, OCH // 2), q * 256:(q + 1) * 256] = _as_u32(
                    stage_o[slot, pl.ds(c * OCH, OCH), q * 256:(q + 1) * 256])
                return wob_v[pl.ds(pl.multiple_of(orow + zsm[0], 8), 8), 0:128]
            tasks.append(task)
        return tasks

    def run_tasks(tch, tasks, done, target, y):
        n = target - done
        for q in range(n):
            r = (q * (y.shape[0] // 8)) // n
            tch = tch + y[8 * r:8 * r + 8, 0:128]
            tok = tasks[done + q]()
            tch = tch + pltpu.bitcast(tok & jnp.uint32(0x3F800000), _F32)
        return tch

    qscale = float(DHA) ** -0.5 * _LOG2E
    npc = D // PIECE
    npieces = 3 * npc

    def p1_body(i, carry, first=False):
        if first:
            xa_copy(0).wait()
            tasks = []
        else:
            pltpu.make_async_copy(xa_hbm.at[pl.ds(0, MB1)], xa_v.at[pl.ds(0, MB1)], sem_xa(i)).wait()
            slot = lax.rem(i - 1, NSLOT)
            group_wait(i - 1, slot)
            tasks = [t for c in range(GCH) for t in relayout_tasks(i - 1, slot, c)]
        r0 = pl.multiple_of(i * MB1, MB1)
        x = xa_v[pl.ds(r0, MB1), :]
        tch = jnp.zeros((8, 128), _F32)
        done = 0
        for p in range(npieces):
            j, n = P1_ORDER[p // npc], p % npc
            if first and n == 0:
                wqkv_copy(j).wait()
            cols = slice(n * PIECE, (n + 1) * PIECE)
            y = _dot(x, wqkv_v[:, j * D + n * PIECE:j * D + (n + 1) * PIECE])
            if not first:
                target = (len(tasks) * (p + 1) + npieces - 1) // npieces
                tch = run_tasks(tch, tasks, done, target, y)
                done = target
            rows_t = slice(n * PIECE // 2, (n + 1) * PIECE // 2)
            if j == 0:
                qT[rows_t, pl.ds(r0, MB1)] = _as_u32((y * qscale).astype(_BF).T)
            elif j == 1:
                kA[pl.ds(pl.multiple_of(i * (MB1 // 2), MB1 // 2), MB1 // 2), cols] = _as_u32(y.astype(_BF))
            else:
                vT[rows_t, pl.ds(r0, MB1)] = _as_u32(y.astype(_BF).T)
        if not first:
            o_scr[0:8, 0:128] = tch

            @pl.when(i - 1 + NSLOT < NGRP)
            def _():
                group_start(i - 1 + NSLOT, slot)

            @pl.when(i == 5)
            def _():
                xb_copy.start()

            @pl.when(i == n_mb - 1)
            def _():
                woa_copy.start()
        return carry

    p1_body(0, 0, first=True)
    lax.fori_loop(1, n_mb, p1_body, 0)

    rowg = lax.broadcasted_iota(jnp.int32, (64, QT), 0) // 16

    def load_qm(u):
        qt = u >> 5
        h = u & (HA - 1)
        qg = qT[pl.ds(pl.multiple_of((h >> 2) * 64, 64), 64), pl.ds(pl.multiple_of(qt * QT, QT), QT)]
        return _as_bf16(jnp.where(rowg == (h & 3), qg, jnp.uint32(0)))

    def scores_blk(u, qm, kb, s_ref, m8):
        g = (u & (HA - 1)) >> 2
        kk = _as_bf16(kA[pl.ds(kb * (KB // 2), KB // 2), pl.ds(pl.multiple_of(g * 128, 128), 128)])
        s = _dot(kk, qm)
        s_ref[pl.ds(kb * KB, KB), :] = s
        mm = jnp.max(s.reshape(KB // 8, 8, QT), axis=0)
        return s, (mm if m8 is None else jnp.maximum(m8, mm))

    def softmax_pv_blk(u, m, kb, s_ref, l8, acc):
        h = u & (HA - 1)
        p = jnp.exp2(s_ref[pl.ds(kb * KB, KB), :] - m)
        ls = jnp.sum(p.reshape(KB // 8, 8, QT), axis=0)
        l8 = ls if l8 is None else l8 + ls
        vt = _as_bf16(vT[pl.ds(pl.multiple_of(h * 16, 16), 16), pl.ds(kb * KB, KB)])
        pv = _dot(vt, p.astype(_BF))
        return l8, (pv if acc is None else acc + pv)

    def finish(u, l8, acc):
        qt = u >> 5
        h = u & (HA - 1)
        r = _recip(jnp.sum(l8, axis=0, keepdims=True))
        oT[pl.ds(pl.multiple_of(h * 16, 16), 16), pl.ds(pl.multiple_of(qt * QT, QT), QT)] = (
            _as_u32((acc * r).astype(_BF)))

    def scores_all(u, s_ref, tasks):
        qm = load_qm(u)
        m8 = None
        tch = jnp.zeros((8, 128), _F32)
        done = 0
        for kb in range(NKB):
            s, m8 = scores_blk(u, qm, kb, s_ref, m8)
            target = (len(tasks) * (kb + 1) + NKB - 1) // NKB
            tch = run_tasks(tch, tasks, done, target, s)
            done = target
        o_scr[8:16, 0:128] = tch
        return jnp.max(m8, axis=0, keepdims=True)

    class Unit:
        def __init__(self, u, m, s_ref, prefetch):
            self.u, self.m, self.s, self.prefetch = u, m, s_ref, prefetch
            self.qm = self.m8 = self.l8 = self.acc = self.m_next = None
            self.kb = 0

        def block(self):
            if self.kb == 0 and self.prefetch:
                self.qm = load_qm(self.u + 2)
            self.l8, self.acc = softmax_pv_blk(self.u, self.m, self.kb, self.s, self.l8, self.acc)
            if self.prefetch:
                _, self.m8 = scores_blk(self.u + 2, self.qm, self.kb, self.s, self.m8)
            self.kb += 1
            if self.kb == NKB:
                finish(self.u, self.l8, self.acc)
                if self.prefetch:
                    self.m_next = jnp.max(self.m8, axis=0, keepdims=True)

    gl = NGRP - 1
    group_wait(gl, gl % NSLOT)
    ptasks = [t for c in range(GCH) for t in relayout_tasks(gl, gl % NSLOT, c)]
    m_a = scores_all(0, s0, ptasks[:len(ptasks) // 2])
    m_b = scores_all(1, s1, ptasks[len(ptasks) // 2:])
    xb_copy.wait()
    mem_copy.wait()

    ri = lax.broadcasted_iota(jnp.int32, (LB, LB), 0)
    ci = lax.broadcasted_iota(jnp.int32, (LB, LB), 1)
    bmask = (ri < MEM) | (ri >= ci)
    bscale = float(DHB) ** -0.5 * _LOG2E
    NG = HB // GB

    def outb_copy(i):
        r0 = pl.multiple_of(i * SEG, SEG)
        return pltpu.make_async_copy(outb_v.at[pl.ds(r0, SEG)], out_hbm.at[pl.ds(r0, SEG), pl.ds(D, D)],
                                     sem_out(1))

    def p2_body(i, carry, last=False):
        mem, ma, mb = carry
        units = [Unit(2 * i, ma, s0, not last), Unit(2 * i + 1, mb, s1, not last)]
        ablocks = [u for u in units for _ in range(NKB)]
        per_tick = len(ablocks) / (2 * TICKS[0] + NG * (TICKS[1] + TICKS[2] + TICKS[3]) + TICKS[4])
        state = {"pos": 0, "credit": 0.0}

        def emit_a(n):
            for _ in range(n):
                if state["pos"] < len(ablocks):
                    ablocks[state["pos"]].block()
                    state["pos"] += 1

        def tick(w):
            state["credit"] += per_tick * w
            n = int(state["credit"] + 1e-6)
            state["credit"] -= n
            emit_a(n)

        r0 = pl.multiple_of(i * SEG, SEG)
        h = jnp.concatenate([mem, xb_v[pl.ds(r0, SEG), :].astype(_F32)], axis=0)

        def proj(j, g):
            w = jnp.concatenate([_as_bf16(wB[j * HB + g * GB + t]) for t in range(GB)], axis=1)
            y = _dot(h, w)
            return y if j == 0 else y.astype(_BF)

        def b_scores(q, k, t):
            sl = slice(t * DHB, (t + 1) * DHB)
            s = jnp.where(bmask, _dot(q[:, sl], k[:, sl], _NT), -1e9)
            mx = jnp.max(s, axis=1, keepdims=True)
            p = jnp.exp2((s - mx) * bscale)
            return p, jnp.sum(p, axis=1, keepdims=True)

        def b_pv(g, t, p, l, v):
            o = _dot(p, v[:, t * DHB:(t + 1) * DHB])
            c0 = (g * GB + t) * DHB
            o_scr[:, c0:c0 + DHB] = _round_bf16(o * _recip(l))

        cur = []
        for j in range(3):
            cur.append(proj(j, 0))
            if j < 2:
                tick(TICKS[0])
        for g in range(NG):
            more = g + 1 < NG
            nxt, pls, half = [], [], GB // 2
            if more:
                nxt.append(proj(0, g + 1))
            for t in range(GB):
                pls.append(b_scores(cur[0], cur[1], t))
            tick(TICKS[1])
            if more:
                nxt.append(proj(1, g + 1))
            for t in range(half):
                b_pv(g, t, *pls[t], cur[2])
            tick(TICKS[2])
            if more:
                nxt.append(proj(2, g + 1))
            for t in range(half, GB):
                b_pv(g, t, *pls[t], cur[2])
            tick(TICKS[3])
            cur = nxt
        acc = _dot(o_scr[...], _as_bf16(wob_v[...]))
        tick(TICKS[4])
        outb_v[pl.ds(r0, SEG), :] = acc[MEM:, :].astype(_BF)
        outb_copy(i).start()
        mem = _round_bf16(acc[:MEM, :])
        emit_a(len(ablocks))
        if last:
            return None
        return (mem, units[0].m_next, units[1].m_next)

    n_it = S // SEG
    carry = lax.fori_loop(0, n_it - 1, p2_body, (mem_v[...].astype(_F32), m_a, m_b))
    p2_body(n_it - 1, carry, last=True)

    woa_copy.wait()

    def outa_copy(i):
        r0 = pl.multiple_of(i * MB3, MB3)
        return pltpu.make_async_copy(xa_v.at[pl.ds(r0, MB3)], out_hbm.at[pl.ds(r0, MB3), pl.ds(0, D)],
                                     sem_out(0))

    def p3_body(i, carry):
        r0 = pl.multiple_of(i * MB3, MB3)
        o = _dot(_as_bf16(oT[:, pl.ds(r0, MB3)]), woa_v[...], _TN)
        xa_v[pl.ds(r0, MB3), :] = o.astype(_BF)
        outa_copy(i).start()
        return carry

    lax.fori_loop(0, S // MB3, p3_body, 0)

    pltpu.make_async_copy(xa_v, out_hbm.at[:, pl.ds(0, D)], sem_out(0)).wait()
    pltpu.make_async_copy(outb_v, out_hbm.at[:, pl.ds(D, D)], sem_out(1)).wait()


@functools.partial(jax.jit, static_argnames=("B_seg_len",))
def pallas_concat_heads__softmax_full_mha__memory_aug_recurrent_mem_tr__prompt_kernel(
    A_x, A_wqkv, A_wo, B_x, B_mem0, B_Wq, B_Wk, B_Wv, B_Wo, B_seg_len,
):
    assert A_x.shape == (1, S, D) and A_wqkv.shape == (D, 3 * D) and A_wo.shape == (D, D)
    assert B_x.shape == (1, S, D) and B_mem0.shape == (1, MEM, D)
    assert B_Wq.shape == B_Wk.shape == B_Wv.shape == (D, HB, DHB) and B_Wo.shape == (HB, DHB, D)
    assert int(B_seg_len) == SEG

    any_spec = pl.BlockSpec(memory_space=pl.ANY)
    scratch = [
        pltpu.VMEM((D, 3 * D), _BF),
        pltpu.VMEM((S, D), _BF),
        pltpu.VMEM((D // 2, S), _U32),
        pltpu.VMEM((S // 2, D), _U32),
        pltpu.VMEM((D // 2, S), _U32),
        pltpu.VMEM((S, QT), _F32),
        pltpu.VMEM((S, QT), _F32),
        pltpu.VMEM((D // 2, S), _U32),
        pltpu.VMEM((D, D), _BF),
        pltpu.VMEM((3 * NSLOT, DG, HB, DHB), _BF),
        pltpu.VMEM((NSLOT, OG, D), _BF),
        pltpu.VMEM((3 * HB, D // 2, DHB), _U32),
        pltpu.VMEM((HB * DHB // 2, D), _U32),
        pltpu.VMEM((S, D), _BF),
        pltpu.VMEM((MEM, D), _BF),
        pltpu.VMEM((LB, HB * DHB), _F32),
        pltpu.VMEM((S, D), _BF),
        pltpu.SMEM((1,), jnp.int32),
        pltpu.SemaphoreType.DMA((NSEM,)),
    ]
    out = pl.pallas_call(
        _kernel,
        out_shape=jax.ShapeDtypeStruct((S, 2 * D), _BF),
        in_specs=[any_spec] * 9,
        out_specs=any_spec,
        scratch_shapes=scratch,
        compiler_params=pltpu.CompilerParams(vmem_limit_bytes=118 * 1024 * 1024),
        name="concat_mha_rmt",
    )(A_x.reshape(S, D), A_wqkv, A_wo, B_x.reshape(S, D), B_mem0.reshape(MEM, D),
      B_Wq, B_Wk, B_Wv, B_Wo.reshape(HB * DHB, D))
    return out.reshape(1, S, 2 * D)
```

```python
import functools

import jax
import jax.numpy as jnp
from jax import lax
from jax.experimental import pallas as pl
from jax.experimental.pallas import tpu as pltpu

_LOG2E = 1.4426950408889634
_NN = (((1,), (0,)), ((), ()))
_NT = (((1,), (1,)), ((), ()))
_TN = (((0,), (0,)), ((), ()))
_BF = jnp.bfloat16
_F32 = jnp.float32
_U32 = jnp.uint32


def _dot(a, b, dims=_NN):
    return lax.dot_general(a, b, dims, preferred_element_type=_F32)


def _as_bf16(u):
    return pltpu.bitcast(u, _BF)


def _as_u32(b):
    return pltpu.bitcast(b, _U32)


def _round_bf16(x):
    return x.astype(_BF).astype(_F32)


def _recip(l):
    r0 = pltpu.reciprocal(l, approx=True)
    return r0 * (2.0 - l * r0)


S = 2048
D = 1024
HA, DHA = 32, 32
HB, DHB = 32, 128
MEM = 8
SEG = 32
LB = MEM + SEG

MB1 = 256
PIECE = 128
MB3 = 128
U3 = 4
QT = 512
KB = 128
NKB = S // KB
NUNITS = HA * (S // QT)
GB = 2
TICKS = (1, 2, 0, 1, 8)
OSPLIT = 2
DCH = 16
NGRP = S // MB1
GCH = D // DCH // NGRP
DG = DCH * GCH
OCH = HB * DHB // (D // DCH)
OG = OCH * GCH
NSLOT = 3
WCH = (256, 768, 1024, 1024)
RELAY_FROM = 8

SEM_XA = 0
SEM_WQKV = SEM_XA + S // MB1
SEM_MISC = SEM_WQKV + len(WCH)
SEM_STAGE = SEM_MISC + 3
SEM_OUT = SEM_STAGE + 4 * NSLOT
NSEM = SEM_OUT + 2


def _kernel(xa_hbm, wqkv_hbm, woa_hbm, xb_hbm, mem_hbm, wq_hbm, wk_hbm, wv_hbm, wob_hbm,
            out_hbm,
            wqkv_v, xa_v, qT, kA, vT, s0, s1, oT, woa_v,
            stage, stage_o, wB, wob_v, xb_v, mem_v, o_scr, outb_v, zsm,
            sems):
    n_mb = S // MB1
    sem_xa = lambda i: sems.at[SEM_XA + i]
    sem_wqkv = lambda j: sems.at[SEM_WQKV + j]
    sem_misc = lambda j: sems.at[SEM_MISC + j]
    sem_stage = lambda j: sems.at[SEM_STAGE + j]
    sem_out = lambda j: sems.at[SEM_OUT + j]
    zsm[0] = 0

    def xa_copy(i):
        return pltpu.make_async_copy(xa_hbm.at[pl.ds(i * MB1, MB1)], xa_v.at[pl.ds(i * MB1, MB1)],
                                     sem_xa(i))

    P1_ORDER = (0, 2, 1)
    wch_cols, pos = [], 0
    for w in WCH:
        wch_cols.append((P1_ORDER[pos // D] * D + pos % D, w))
        pos += w

    def wqkv_copy(c):
        c0, w = wch_cols[c]
        return pltpu.make_async_copy(wqkv_hbm.at[:, pl.ds(c0, w)], wqkv_v.at[:, pl.ds(c0, w)], sem_wqkv(c))

    woa_copy = pltpu.make_async_copy(woa_hbm, woa_v, sem_misc(0))
    xb_copy = pltpu.make_async_copy(xb_hbm, xb_v, sem_misc(1))
    mem_copy = pltpu.make_async_copy(mem_hbm, mem_v, sem_misc(2))
    wsrc = (wq_hbm, wk_hbm, wv_hbm)

    def stage_copy(g, slot, j):
        sem = sem_stage(slot * 4 + j)
        if j == 3:
            return pltpu.make_async_copy(wob_hbm.at[pl.ds(g * OG, OG)], stage_o.at[slot], sem)
        return pltpu.make_async_copy(wsrc[j].at[pl.ds(g * DG, DG)], stage.at[slot * 3 + j], sem)

    def group_start(g, slot):
        for j in range(4):
            stage_copy(g, slot, j).start()

    def group_wait(g, slot):
        for j in range(4):
            stage_copy(g, slot, j).wait()

    xa_copy(0).start()
    for c in range(len(WCH)):
        wqkv_copy(c).start()
    xa_copy(1).start()
    group_start(0, 0)
    xa_copy(2).start()
    group_start(1, 1)
    xa_copy(3).start()
    group_start(2, 2)
    for i in range(4, n_mb):
        xa_copy(i).start()
    mem_copy.start()

    j_iota = lax.broadcasted_iota(jnp.int32, (8, 128), 0)

    def relayout_tasks(g, slot, c):
        row = pl.multiple_of(g * (DG // 2) + c * 8, 8)
        tasks = []
        for j in range(3):
            for g2 in range(2):
                for odd in range(2):
                    def task(j=j, g2=g2, odd=odd):
                        X = []
                        for i in range(8):
                            a = _as_u32(stage[slot * 3 + j, c * DCH + 2 * i, g2 * 16:(g2 + 1) * 16, :])
                            b = _as_u32(stage[slot * 3 + j, c * DCH + 2 * i + 1, g2 * 16:(g2 + 1) * 16, :])
                            if odd == 0:
                                X.append((a & jnp.uint32(0xFFFF)) | (b << 16))
                            else:
                                X.append((a >> 16) | (b & jnp.uint32(0xFFFF0000)))
                        for s in (4, 2, 1):
                            mask = (j_iota & s) == 0
                            for i in range(8):
                                if i & s:
                                    continue
                                x, y = X[i], X[i + s]
                                X[i] = jnp.where(mask, x, pltpu.roll(y, s, 0))
                                X[i + s] = jnp.where(mask, pltpu.roll(x, 8 - s, 0), y)
                        for jj in range(8):
                            wB[j * HB + g2 * 16 + 2 * jj + odd, pl.ds(row, 8), :] = X[jj]
                        return wB[zsm[0], pl.ds(row, 8), :]
                    tasks.append(task)
        orow = pl.multiple_of(g * (OG // 2) + c * (OCH // 2), OCH // 2)
        for q in range(4):
            def task(q=q):
                wob_v[pl.ds(orow, OCH // 2), q * 256:(q + 1) * 256] = _as_u32(
                    stage_o[slot, pl.ds(c * OCH, OCH), q * 256:(q + 1) * 256])
                return wob_v[pl.ds(pl.multiple_of(orow + zsm[0], 8), 8), 0:128]
            tasks.append(task)
        return tasks

    def run_tasks(tch, tasks, done, target, y):
        n = target - done
        for q in range(n):
            r = (q * (y.shape[0] // 8)) // n
            tch = tch + y[8 * r:8 * r + 8, 0:128]
            tok = tasks[done + q]()
            tch = tch + pltpu.bitcast(tok & jnp.uint32(0x3F800000), _F32)
        return tch

    qscale = float(DHA) ** -0.5 * _LOG2E
    npc = D // PIECE
    npieces = 3 * npc

    def p1_body(i, carry, first=False):
        if first:
            xa_copy(0).wait()
            tasks = []
        else:
            pltpu.make_async_copy(xa_hbm.at[pl.ds(0, MB1)], xa_v.at[pl.ds(0, MB1)], sem_xa(i)).wait()
            slot = lax.rem(i - 1, NSLOT)
            tasks = [t for c in range(GCH) for t in relayout_tasks(i - 1, slot, c)]
        r0 = pl.multiple_of(i * MB1, MB1)
        x = xa_v[pl.ds(r0, MB1), :]
        tch = jnp.zeros((8, 128), _F32)
        done = 0
        for p in range(npieces):
            j, n = P1_ORDER[p // npc], p % npc
            if first:
                for c, (c0, _) in enumerate(wch_cols):
                    if c0 == j * D + n * PIECE:
                        wqkv_copy(c).wait()
            cols = slice(n * PIECE, (n + 1) * PIECE)
            y = _dot(x, wqkv_v[:, j * D + n * PIECE:j * D + (n + 1) * PIECE])
            if not first:
                if p == RELAY_FROM:
                    group_wait(i - 1, slot)
                active = npieces - RELAY_FROM
                target = max(0, (len(tasks) * (p + 1 - RELAY_FROM) + active - 1) // active)
                if target == done:
                    tch = tch + y[0:8, 0:128]
                tch = run_tasks(tch, tasks, done, target, y)
                done = target
            rows_t = slice(n * PIECE // 2, (n + 1) * PIECE // 2)
            if j == 0:
                qT[rows_t, pl.ds(r0, MB1)] = _as_u32((y * qscale).astype(_BF).T)
            elif j == 1:
                kA[pl.ds(pl.multiple_of(i * (MB1 // 2), MB1 // 2), MB1 // 2), cols] = _as_u32(y.astype(_BF))
            else:
                vT[rows_t, pl.ds(r0, MB1)] = _as_u32(y.astype(_BF).T)
        if not first:
            o_scr[0:8, 0:128] = tch

            @pl.when(i - 1 + NSLOT < NGRP)
            def _():
                group_start(i - 1 + NSLOT, slot)

            @pl.when(i == 5)
            def _():
                xb_copy.start()

            @pl.when(i == n_mb - 1)
            def _():
                woa_copy.start()
        return carry

    p1_body(0, 0, first=True)
    lax.fori_loop(1, n_mb, p1_body, 0)

    rowg = lax.broadcasted_iota(jnp.int32, (64, QT), 0) // 16

    def load_qm(u):
        qt = u >> 5
        h = u & (HA - 1)
        qg = qT[pl.ds(pl.multiple_of((h >> 2) * 64, 64), 64), pl.ds(pl.multiple_of(qt * QT, QT), QT)]
        return _as_bf16(jnp.where(rowg == (h & 3), qg, jnp.uint32(0)))

    def scores_blk(u, qm, kb, s_ref, m8):
        g = (u & (HA - 1)) >> 2
        kk = _as_bf16(kA[pl.ds(kb * (KB // 2), KB // 2), pl.ds(pl.multiple_of(g * 128, 128), 128)])
        s = _dot(kk, qm)
        s_ref[pl.ds(kb * KB, KB), :] = s
        mm = jnp.max(s.reshape(KB // 8, 8, QT), axis=0)
        return s, (mm if m8 is None else jnp.maximum(m8, mm))

    def softmax_pv_blk(u, m, kb, s_ref, l8, acc):
        h = u & (HA - 1)
        p = jnp.exp2(s_ref[pl.ds(kb * KB, KB), :] - m)
        ls = jnp.sum(p.reshape(KB // 8, 8, QT), axis=0)
        l8 = ls if l8 is None else l8 + ls
        vt = _as_bf16(vT[pl.ds(pl.multiple_of(h * 16, 16), 16), pl.ds(kb * KB, KB)])
        pv = _dot(vt, p.astype(_BF))
        return l8, (pv if acc is None else acc + pv)

    def finish(u, l8, acc):
        qt = u >> 5
        h = u & (HA - 1)
        r = _recip(jnp.sum(l8, axis=0, keepdims=True))
        oT[pl.ds(pl.multiple_of(h * 16, 16), 16), pl.ds(pl.multiple_of(qt * QT, QT), QT)] = (
            _as_u32((acc * r).astype(_BF)))

    def scores_all(u, s_ref, tasks):
        qm = load_qm(u)
        m8 = None
        tch = jnp.zeros((8, 128), _F32)
        done = 0
        for kb in range(NKB):
            s, m8 = scores_blk(u, qm, kb, s_ref, m8)
            target = (len(tasks) * (kb + 1) + NKB - 1) // NKB
            tch = run_tasks(tch, tasks, done, target, s)
            done = target
        o_scr[8:16, 0:128] = tch
        return jnp.max(m8, axis=0, keepdims=True)

    class Unit:
        def __init__(self, u, m, s_ref, prefetch):
            self.u, self.m, self.s, self.prefetch = u, m, s_ref, prefetch
            self.qm = self.m8 = self.l8 = self.acc = self.m_next = None
            self.kb = 0

        def block(self):
            if self.kb == 0 and self.prefetch:
                self.qm = load_qm(self.u + 2)
            self.l8, self.acc = softmax_pv_blk(self.u, self.m, self.kb, self.s, self.l8, self.acc)
            if self.prefetch:
                _, self.m8 = scores_blk(self.u + 2, self.qm, self.kb, self.s, self.m8)
            self.kb += 1
            if self.kb == NKB:
                finish(self.u, self.l8, self.acc)
                if self.prefetch:
                    self.m_next = jnp.max(self.m8, axis=0, keepdims=True)

    gl = NGRP - 1
    group_wait(gl, gl % NSLOT)
    ptasks = [t for c in range(GCH) for t in relayout_tasks(gl, gl % NSLOT, c)]
    m_a = scores_all(0, s0, ptasks[:len(ptasks) // 2])
    m_b = scores_all(1, s1, ptasks[len(ptasks) // 2:])
    xb_copy.wait()
    mem_copy.wait()

    ri = lax.broadcasted_iota(jnp.int32, (LB, LB), 0)
    ci = lax.broadcasted_iota(jnp.int32, (LB, LB), 1)
    bmask = (ri < MEM) | (ri >= ci)
    bscale = float(DHB) ** -0.5 * _LOG2E
    NG = HB // GB

    def outb_copy(i):
        r0 = pl.multiple_of(i * SEG, SEG)
        return pltpu.make_async_copy(outb_v.at[pl.ds(r0, SEG)], out_hbm.at[pl.ds(r0, SEG), pl.ds(D, D)],
                                     sem_out(1))

    def p2_body(i, carry, last=False):
        mem, ma, mb = carry
        units = [Unit(2 * i, ma, s0, not last), Unit(2 * i + 1, mb, s1, not last)]
        ablocks = [u for u in units for _ in range(NKB)]
        per_tick = len(ablocks) / (2 * TICKS[0] + NG * (TICKS[1] + TICKS[2] + TICKS[3]) + TICKS[4])
        state = {"pos": 0, "credit": 0.0}

        def emit_a(n):
            for _ in range(n):
                if state["pos"] < len(ablocks):
                    ablocks[state["pos"]].block()
                    state["pos"] += 1

        def tick(w):
            state["credit"] += per_tick * w
            n = int(state["credit"] + 1e-6)
            state["credit"] -= n
            emit_a(n)

        r0 = pl.multiple_of(i * SEG, SEG)
        h = jnp.concatenate([mem, xb_v[pl.ds(r0, SEG), :].astype(_F32)], axis=0)

        def proj(j, g):
            w = jnp.concatenate([_as_bf16(wB[j * HB + g * GB + t]) for t in range(GB)], axis=1)
            y = _dot(h, w)
            return y if j == 0 else y.astype(_BF)

        def b_scores(q, k, t):
            sl = slice(t * DHB, (t + 1) * DHB)
            s = jnp.where(bmask, _dot(q[:, sl], k[:, sl], _NT), -1e9)
            mx = jnp.max(s, axis=1, keepdims=True)
            p = jnp.exp2((s - mx) * bscale)
            return p, jnp.sum(p, axis=1, keepdims=True)

        def b_pv(g, t, p, l, v):
            o = _dot(p, v[:, t * DHB:(t + 1) * DHB])
            c0 = (g * GB + t) * DHB
            o_scr[:, c0:c0 + DHB] = _round_bf16(o * _recip(l))

        cur = []
        for j in range(3):
            cur.append(proj(j, 0))
            if j < 2:
                tick(TICKS[0])
        for g in range(NG):
            more = g + 1 < NG
            nxt, pls, half = [], [], GB // 2
            if more:
                nxt.append(proj(0, g + 1))
            for t in range(GB):
                pls.append(b_scores(cur[0], cur[1], t))
            tick(TICKS[1])
            if more:
                nxt.append(proj(1, g + 1))
            for t in range(half):
                b_pv(g, t, *pls[t], cur[2])
            tick(TICKS[2])
            if more:
                nxt.append(proj(2, g + 1))
            for t in range(half, GB):
                b_pv(g, t, *pls[t], cur[2])
            tick(TICKS[3])
            cur = nxt
        parts, nw = [], D // OSPLIT
        for q in range(OSPLIT):
            parts.append(_dot(o_scr[...], _as_bf16(wob_v[:, q * nw:(q + 1) * nw])))
            tick(TICKS[4] / OSPLIT)
        acc = jnp.concatenate(parts, axis=1)
        outb_v[pl.ds(r0, SEG), :] = acc[MEM:, :].astype(_BF)
        outb_copy(i).start()
        mem = _round_bf16(acc[:MEM, :])
        emit_a(len(ablocks))
        if last:
            return None
        return (mem, units[0].m_next, units[1].m_next)

    n_it = S // SEG
    carry = lax.fori_loop(0, n_it - 1, p2_body, (mem_v[...].astype(_F32), m_a, m_b))
    p2_body(n_it - 1, carry, last=True)

    woa_copy.wait()

    def outa_copy(i):
        r0 = pl.multiple_of(i * MB3, MB3)
        return pltpu.make_async_copy(xa_v.at[pl.ds(r0, MB3)], out_hbm.at[pl.ds(r0, MB3), pl.ds(0, D)],
                                     sem_out(0))

    def p3_body(i2, carry):
        for u in range(U3):
            i = i2 * U3 + u
            r0 = pl.multiple_of(i * MB3, MB3)
            o = _dot(_as_bf16(oT[:, pl.ds(r0, MB3)]), woa_v[...], _TN)
            xa_v[pl.ds(r0, MB3), :] = o.astype(_BF)
            outa_copy(i).start()
        return carry

    lax.fori_loop(0, S // (MB3 * U3), p3_body, 0)

    pltpu.make_async_copy(xa_v, out_hbm.at[:, pl.ds(0, D)], sem_out(0)).wait()
    pltpu.make_async_copy(outb_v, out_hbm.at[:, pl.ds(D, D)], sem_out(1)).wait()


@functools.partial(jax.jit, static_argnames=("B_seg_len",))
def pallas_concat_heads__softmax_full_mha__memory_aug_recurrent_mem_tr__prompt_kernel(
    A_x, A_wqkv, A_wo, B_x, B_mem0, B_Wq, B_Wk, B_Wv, B_Wo, B_seg_len,
):
    assert A_x.shape == (1, S, D) and A_wqkv.shape == (D, 3 * D) and A_wo.shape == (D, D)
    assert B_x.shape == (1, S, D) and B_mem0.shape == (1, MEM, D)
    assert B_Wq.shape == B_Wk.shape == B_Wv.shape == (D, HB, DHB) and B_Wo.shape == (HB, DHB, D)
    assert int(B_seg_len) == SEG

    any_spec = pl.BlockSpec(memory_space=pl.ANY)
    scratch = [
        pltpu.VMEM((D, 3 * D), _BF),
        pltpu.VMEM((S, D), _BF),
        pltpu.VMEM((D // 2, S), _U32),
        pltpu.VMEM((S // 2, D), _U32),
        pltpu.VMEM((D // 2, S), _U32),
        pltpu.VMEM((S, QT), _F32),
        pltpu.VMEM((S, QT), _F32),
        pltpu.VMEM((D // 2, S), _U32),
        pltpu.VMEM((D, D), _BF),
        pltpu.VMEM((3 * NSLOT, DG, HB, DHB), _BF),
        pltpu.VMEM((NSLOT, OG, D), _BF),
        pltpu.VMEM((3 * HB, D // 2, DHB), _U32),
        pltpu.VMEM((HB * DHB // 2, D), _U32),
        pltpu.VMEM((S, D), _BF),
        pltpu.VMEM((MEM, D), _BF),
        pltpu.VMEM((LB, HB * DHB), _F32),
        pltpu.VMEM((S, D), _BF),
        pltpu.SMEM((1,), jnp.int32),
        pltpu.SemaphoreType.DMA((NSEM,)),
    ]
    out = pl.pallas_call(
        _kernel,
        out_shape=jax.ShapeDtypeStruct((S, 2 * D), _BF),
        in_specs=[any_spec] * 9,
        out_specs=any_spec,
        scratch_shapes=scratch,
        compiler_params=pltpu.CompilerParams(vmem_limit_bytes=118 * 1024 * 1024),
        name="concat_mha_rmt",
    )(A_x.reshape(S, D), A_wqkv, A_wo, B_x.reshape(S, D), B_mem0.reshape(MEM, D),
      B_Wq, B_Wk, B_Wv, B_Wo.reshape(HB * DHB, D))
    return out.reshape(1, S, 2 * D)
```

```python
import functools

import jax
import jax.numpy as jnp
from jax import lax
from jax.experimental import pallas as pl
from jax.experimental.pallas import tpu as pltpu

_LOG2E = 1.4426950408889634
_NN = (((1,), (0,)), ((), ()))
_NT = (((1,), (1,)), ((), ()))
_TN = (((0,), (0,)), ((), ()))
_BF = jnp.bfloat16
_F32 = jnp.float32
_U32 = jnp.uint32


def _dot(a, b, dims=_NN):
    return lax.dot_general(a, b, dims, preferred_element_type=_F32)


def _as_bf16(u):
    return pltpu.bitcast(u, _BF)


def _as_u32(b):
    return pltpu.bitcast(b, _U32)


def _round_bf16(x):
    return x.astype(_BF).astype(_F32)


def _recip(l):
    r0 = pltpu.reciprocal(l, approx=True)
    return r0 * (2.0 - l * r0)


S = 2048
D = 1024
HA, DHA = 32, 32
HB, DHB = 32, 128
MEM = 8
SEG = 32
LB = MEM + SEG

MB1 = 256
PIECE = 128
MB3 = 128
U3 = 4
QT = 512
KB = 128
NKB = S // KB
NUNITS = HA * (S // QT)
GB = 2
TICKS = (1, 2, 0, 1, 8)
OSPLIT = 4
DCH = 16
NGRP = S // MB1
GCH = D // DCH // NGRP
DG = DCH * GCH
OCH = HB * DHB // (D // DCH)
OG = OCH * GCH
NSLOT = 3
WCH = (256, 768, 1024, 1024)
RELAY_FROM = 8

SEM_XA = 0
SEM_WQKV = SEM_XA + S // MB1
SEM_MISC = SEM_WQKV + len(WCH)
SEM_STAGE = SEM_MISC + 3
SEM_OUT = SEM_STAGE + 4 * NSLOT
NSEM = SEM_OUT + 2


def _kernel(xa_hbm, wqkv_hbm, woa_hbm, xb_hbm, mem_hbm, wq_hbm, wk_hbm, wv_hbm, wob_hbm,
            out_hbm,
            wqkv_v, xa_v, qT, kA, vT, s0, s1, oT, woa_v,
            stage, stage_o, wB, wob_v, xb_v, mem_v, o_scr, outb_v, zsm,
            sems):
    n_mb = S // MB1
    sem_xa = lambda i: sems.at[SEM_XA + i]
    sem_wqkv = lambda j: sems.at[SEM_WQKV + j]
    sem_misc = lambda j: sems.at[SEM_MISC + j]
    sem_stage = lambda j: sems.at[SEM_STAGE + j]
    sem_out = lambda j: sems.at[SEM_OUT + j]
    zsm[0] = 0

    def xa_copy(i):
        return pltpu.make_async_copy(xa_hbm.at[pl.ds(i * MB1, MB1)], xa_v.at[pl.ds(i * MB1, MB1)],
                                     sem_xa(i))

    P1_ORDER = (0, 2, 1)
    wch_cols, pos = [], 0
    for w in WCH:
        wch_cols.append((P1_ORDER[pos // D] * D + pos % D, w))
        pos += w

    def wqkv_copy(c):
        c0, w = wch_cols[c]
        return pltpu.make_async_copy(wqkv_hbm.at[:, pl.ds(c0, w)], wqkv_v.at[:, pl.ds(c0, w)], sem_wqkv(c))

    woa_copy = pltpu.make_async_copy(woa_hbm, woa_v, sem_misc(0))
    xb_copy = pltpu.make_async_copy(xb_hbm, xb_v, sem_misc(1))
    mem_copy = pltpu.make_async_copy(mem_hbm, mem_v, sem_misc(2))
    wsrc = (wq_hbm, wk_hbm, wv_hbm)

    def stage_copy(g, slot, j):
        sem = sem_stage(slot * 4 + j)
        if j == 3:
            return pltpu.make_async_copy(wob_hbm.at[pl.ds(g * OG, OG)], stage_o.at[slot], sem)
        return pltpu.make_async_copy(wsrc[j].at[pl.ds(g * DG, DG)], stage.at[slot * 3 + j], sem)

    def group_start(g, slot):
        for j in range(4):
            stage_copy(g, slot, j).start()

    def group_wait(g, slot):
        for j in range(4):
            stage_copy(g, slot, j).wait()

    xa_copy(0).start()
    for c in range(len(WCH)):
        wqkv_copy(c).start()
    xa_copy(1).start()
    group_start(0, 0)
    xa_copy(2).start()
    group_start(1, 1)
    xa_copy(3).start()
    group_start(2, 2)
    for i in range(4, n_mb):
        xa_copy(i).start()
    mem_copy.start()

    j_iota = lax.broadcasted_iota(jnp.int32, (8, 128), 0)

    def relayout_tasks(g, slot, c):
        row = pl.multiple_of(g * (DG // 2) + c * 8, 8)
        tasks = []
        for j in range(3):
            for g2 in range(2):
                for odd in range(2):
                    def task(j=j, g2=g2, odd=odd):
                        X = []
                        for i in range(8):
                            a = _as_u32(stage[slot * 3 + j, c * DCH + 2 * i, g2 * 16:(g2 + 1) * 16, :])
                            b = _as_u32(stage[slot * 3 + j, c * DCH + 2 * i + 1, g2 * 16:(g2 + 1) * 16, :])
                            if odd == 0:
                                X.append((a & jnp.uint32(0xFFFF)) | (b << 16))
                            else:
                                X.append((a >> 16) | (b & jnp.uint32(0xFFFF0000)))
                        for s in (4, 2, 1):
                            mask = (j_iota & s) == 0
                            for i in range(8):
                                if i & s:
                                    continue
                                x, y = X[i], X[i + s]
                                X[i] = jnp.where(mask, x, pltpu.roll(y, s, 0))
                                X[i + s] = jnp.where(mask, pltpu.roll(x, 8 - s, 0), y)
                        for jj in range(8):
                            wB[j * HB + g2 * 16 + 2 * jj + odd, pl.ds(row, 8), :] = X[jj]
                        return wB[zsm[0], pl.ds(row, 8), :]
                    tasks.append(task)
        orow = pl.multiple_of(g * (OG // 2) + c * (OCH // 2), OCH // 2)
        for q in range(4):
            def task(q=q):
                wob_v[pl.ds(orow, OCH // 2), q * 256:(q + 1) * 256] = _as_u32(
                    stage_o[slot, pl.ds(c * OCH, OCH), q * 256:(q + 1) * 256])
                return wob_v[pl.ds(pl.multiple_of(orow + zsm[0], 8), 8), 0:128]
            tasks.append(task)
        return tasks

    def run_tasks(tch, tasks, done, target, y):
        n = target - done
        for q in range(n):
            r = (q * (y.shape[0] // 8)) // n
            tch = tch + y[8 * r:8 * r + 8, 0:128]
            tok = tasks[done + q]()
            tch = tch + pltpu.bitcast(tok & jnp.uint32(0x3F800000), _F32)
        return tch

    qscale = float(DHA) ** -0.5 * _LOG2E
    npc = D // PIECE
    npieces = 3 * npc

    def p1_body(i, carry, first=False):
        if first:
            xa_copy(0).wait()
            tasks = []
        else:
            xa_copy(i).wait()
            slot = lax.rem(i - 1, NSLOT)
            tasks = [t for c in range(GCH) for t in relayout_tasks(i - 1, slot, c)]
        r0 = pl.multiple_of(i * MB1, MB1)
        x = xa_v[pl.ds(r0, MB1), :]
        tch = jnp.zeros((8, 128), _F32)
        done = 0
        for p in range(npieces):
            j, n = P1_ORDER[p // npc], p % npc
            if first:
                for c, (c0, _) in enumerate(wch_cols):
                    if c0 == j * D + n * PIECE:
                        wqkv_copy(c).wait()
            y = _dot(x, wqkv_v[:, j * D + n * PIECE:j * D + (n + 1) * PIECE])
            if not first:
                if p == RELAY_FROM:
                    group_wait(i - 1, slot)
                active = npieces - RELAY_FROM
                target = max(0, (len(tasks) * (p + 1 - RELAY_FROM) + active - 1) // active)
                if target == done:
                    tch = tch + y[0:8, 0:128]
                tch = run_tasks(tch, tasks, done, target, y)
                done = target
            rows_t = slice(n * PIECE // 2, (n + 1) * PIECE // 2)
            if j == 0:
                qT[rows_t, pl.ds(r0, MB1)] = _as_u32((y * qscale).astype(_BF).T)
            elif j == 1:
                yu = _as_u32(y.astype(_BF))
                rows_k = pl.ds(pl.multiple_of(i * (MB1 // 2), MB1 // 2), MB1 // 2)
                for t in range(PIECE // DHA):
                    kA[n * (PIECE // DHA) + t, rows_k, :] = yu[:, t * DHA:(t + 1) * DHA]
            else:
                vT[rows_t, pl.ds(r0, MB1)] = _as_u32(y.astype(_BF).T)
        if not first:
            o_scr[0:8, 0:128] = tch

            @pl.when(i - 1 + NSLOT < NGRP)
            def _():
                group_start(i - 1 + NSLOT, slot)

            @pl.when(i == 5)
            def _():
                xb_copy.start()

            @pl.when(i == n_mb - 1)
            def _():
                woa_copy.start()
        return carry

    p1_body(0, 0, first=True)
    lax.fori_loop(1, n_mb, p1_body, 0)

    def load_qm(u):
        qt = u >> 5
        h = u & (HA - 1)
        return _as_bf16(qT[pl.ds(pl.multiple_of(h * (DHA // 2), DHA // 2), DHA // 2),
                           pl.ds(pl.multiple_of(qt * QT, QT), QT)])

    def scores_blk(u, qm, kb, s_ref, m8):
        kk = _as_bf16(kA[u & (HA - 1), pl.ds(kb * (KB // 2), KB // 2), :])
        s = _dot(kk, qm)
        s_ref[pl.ds(kb * KB, KB), :] = s
        mm = jnp.max(s.reshape(KB // 8, 8, QT), axis=0)
        return s, (mm if m8 is None else jnp.maximum(m8, mm))

    def softmax_pv_blk(u, m, kb, s_ref, l8, acc):
        h = u & (HA - 1)
        p = jnp.exp2(s_ref[pl.ds(kb * KB, KB), :] - m)
        ls = jnp.sum(p.reshape(KB // 8, 8, QT), axis=0)
        l8 = ls if l8 is None else l8 + ls
        vt = _as_bf16(vT[pl.ds(pl.multiple_of(h * 16, 16), 16), pl.ds(kb * KB, KB)])
        pv = _dot(vt, p.astype(_BF))
        return l8, (pv if acc is None else acc + pv)

    def finish(u, l8, acc):
        qt = u >> 5
        h = u & (HA - 1)
        r = _recip(jnp.sum(l8, axis=0, keepdims=True))
        oT[pl.ds(pl.multiple_of(h * 16, 16), 16), pl.ds(pl.multiple_of(qt * QT, QT), QT)] = (
            _as_u32((acc * r).astype(_BF)))

    def scores_all(u, s_ref, tasks):
        qm = load_qm(u)
        m8 = None
        tch = jnp.zeros((8, 128), _F32)
        done = 0
        for kb in range(NKB):
            s, m8 = scores_blk(u, qm, kb, s_ref, m8)
            target = (len(tasks) * (kb + 1) + NKB - 1) // NKB
            tch = run_tasks(tch, tasks, done, target, s)
            done = target
        o_scr[8:16, 0:128] = tch
        return m8

    class Unit:
        def __init__(self, u, m, s_ref, prefetch):
            self.u, self.m, self.s, self.prefetch = u, m, s_ref, prefetch
            self.qm = self.m8 = self.l8 = self.acc = None
            self.kb = 0

        def block(self):
            if self.kb == 0 and self.prefetch:
                self.qm = load_qm(self.u + 2)
            self.l8, self.acc = softmax_pv_blk(self.u, self.m, self.kb, self.s, self.l8, self.acc)
            if self.prefetch:
                _, self.m8 = scores_blk(self.u + 2, self.qm, self.kb, self.s, self.m8)
            self.kb += 1
            if self.kb == NKB:
                finish(self.u, self.l8, self.acc)

    gl = NGRP - 1
    group_wait(gl, gl % NSLOT)
    ptasks = [t for c in range(GCH) for t in relayout_tasks(gl, gl % NSLOT, c)]
    m_a = scores_all(0, s0, ptasks[:len(ptasks) // 2])
    m_b = scores_all(1, s1, ptasks[len(ptasks) // 2:])
    xb_copy.wait()
    mem_copy.wait()

    ri = lax.broadcasted_iota(jnp.int32, (LB, LB), 0)
    ci = lax.broadcasted_iota(jnp.int32, (LB, LB), 1)
    bmask = (ri < MEM) | (ri >= ci)
    bscale = float(DHB) ** -0.5 * _LOG2E
    NG = HB // GB

    def outb_copy(i):
        r0 = pl.multiple_of(i * SEG, SEG)
        return pltpu.make_async_copy(outb_v.at[pl.ds(r0, SEG)], out_hbm.at[pl.ds(r0, SEG), pl.ds(D, D)],
                                     sem_out(1))

    def p2_body(i, carry, last=False):
        mem, ma, mb = carry
        ma = jnp.max(ma, axis=0, keepdims=True)
        mb = jnp.max(mb, axis=0, keepdims=True)
        units = [Unit(2 * i, ma, s0, not last), Unit(2 * i + 1, mb, s1, not last)]
        ablocks = [u for u in units for _ in range(NKB)]
        per_tick = len(ablocks) / (2 * TICKS[0] + NG * (TICKS[1] + TICKS[2] + TICKS[3]) + TICKS[4])
        state = {"pos": 0, "credit": 0.0}

        def emit_a(n):
            for _ in range(n):
                if state["pos"] < len(ablocks):
                    ablocks[state["pos"]].block()
                    state["pos"] += 1

        def tick(w):
            state["credit"] += per_tick * w
            n = int(state["credit"] + 1e-6)
            state["credit"] -= n
            emit_a(n)

        r0 = pl.multiple_of(i * SEG, SEG)
        h = jnp.concatenate([mem, xb_v[pl.ds(r0, SEG), :].astype(_F32)], axis=0)

        def proj(j, g):
            w = jnp.concatenate([_as_bf16(wB[j * HB + g * GB + t]) for t in range(GB)], axis=1)
            y = _dot(h, w)
            return y if j == 0 else y.astype(_BF)

        def b_scores(q, k, t):
            sl = slice(t * DHB, (t + 1) * DHB)
            s = jnp.where(bmask, _dot(q[:, sl], k[:, sl], _NT), -1e9)
            mx = jnp.max(s, axis=1, keepdims=True)
            p = jnp.exp2((s - mx) * bscale)
            return p, jnp.sum(p, axis=1, keepdims=True)

        def b_pv(g, t, p, l, v):
            o = _dot(p, v[:, t * DHB:(t + 1) * DHB])
            c0 = (g * GB + t) * DHB
            o_scr[:, c0:c0 + DHB] = _round_bf16(o * _recip(l))

        cur = []
        for j in range(3):
            cur.append(proj(j, 0))
            if j < 2:
                tick(TICKS[0])
        for g in range(NG):
            more = g + 1 < NG
            nxt, pls, half = [], [], GB // 2
            if more:
                nxt.append(proj(0, g + 1))
            for t in range(GB):
                pls.append(b_scores(cur[0], cur[1], t))
            tick(TICKS[1])
            if more:
                nxt.append(proj(1, g + 1))
            for t in range(half):
                b_pv(g, t, *pls[t], cur[2])
            tick(TICKS[2])
            if more:
                nxt.append(proj(2, g + 1))
            for t in range(half, GB):
                b_pv(g, t, *pls[t], cur[2])
            tick(TICKS[3])
            cur = nxt
        parts, nw = [], D // OSPLIT
        for q in range(OSPLIT):
            parts.append(_dot(o_scr[...], _as_bf16(wob_v[:, q * nw:(q + 1) * nw])))
            tick(TICKS[4] / OSPLIT)
        acc = jnp.concatenate(parts, axis=1)
        outb_v[pl.ds(r0, SEG), :] = acc[MEM:, :].astype(_BF)
        outb_copy(i).start()
        mem = _round_bf16(acc[:MEM, :])
        emit_a(len(ablocks))
        if last:
            return None
        return (mem, units[0].m8, units[1].m8)

    n_it = S // SEG
    carry = lax.fori_loop(0, n_it - 1, p2_body, (mem_v[...].astype(_F32), m_a, m_b))
    p2_body(n_it - 1, carry, last=True)

    woa_copy.wait()

    def outa_copy(i):
        r0 = pl.multiple_of(i * MB3, MB3)
        return pltpu.make_async_copy(xa_v.at[pl.ds(r0, MB3)], out_hbm.at[pl.ds(r0, MB3), pl.ds(0, D)],
                                     sem_out(0))

    def p3_body(i2, carry):
        for u in range(U3):
            i = i2 * U3 + u
            r0 = pl.multiple_of(i * MB3, MB3)
            o = _dot(_as_bf16(oT[:, pl.ds(r0, MB3)]), woa_v[...], _TN)
            xa_v[pl.ds(r0, MB3), :] = o.astype(_BF)
            outa_copy(i).start()
        return carry

    lax.fori_loop(0, S // (MB3 * U3), p3_body, 0)

    pltpu.make_async_copy(xa_v, out_hbm.at[:, pl.ds(0, D)], sem_out(0)).wait()
    pltpu.make_async_copy(outb_v, out_hbm.at[:, pl.ds(D, D)], sem_out(1)).wait()


@functools.partial(jax.jit, static_argnames=("B_seg_len",))
def pallas_concat_heads__softmax_full_mha__memory_aug_recurrent_mem_tr__prompt_kernel(
    A_x, A_wqkv, A_wo, B_x, B_mem0, B_Wq, B_Wk, B_Wv, B_Wo, B_seg_len,
):
    assert A_x.shape == (1, S, D) and A_wqkv.shape == (D, 3 * D) and A_wo.shape == (D, D)
    assert B_x.shape == (1, S, D) and B_mem0.shape == (1, MEM, D)
    assert B_Wq.shape == B_Wk.shape == B_Wv.shape == (D, HB, DHB) and B_Wo.shape == (HB, DHB, D)
    assert int(B_seg_len) == SEG

    any_spec = pl.BlockSpec(memory_space=pl.ANY)
    scratch = [
        pltpu.VMEM((D, 3 * D), _BF),
        pltpu.VMEM((S, D), _BF),
        pltpu.VMEM((D // 2, S), _U32),
        pltpu.VMEM((HA, S // 2, DHA), _U32),
        pltpu.VMEM((D // 2, S), _U32),
        pltpu.VMEM((S, QT), _F32),
        pltpu.VMEM((S, QT), _F32),
        pltpu.VMEM((D // 2, S), _U32),
        pltpu.VMEM((D, D), _BF),
        pltpu.VMEM((3 * NSLOT, DG, HB, DHB), _BF),
        pltpu.VMEM((NSLOT, OG, D), _BF),
        pltpu.VMEM((3 * HB, D // 2, DHB), _U32),
        pltpu.VMEM((HB * DHB // 2, D), _U32),
        pltpu.VMEM((S, D), _BF),
        pltpu.VMEM((MEM, D), _BF),
        pltpu.VMEM((LB, HB * DHB), _F32),
        pltpu.VMEM((S, D), _BF),
        pltpu.SMEM((1,), jnp.int32),
        pltpu.SemaphoreType.DMA((NSEM,)),
    ]
    out = pl.pallas_call(
        _kernel,
        out_shape=jax.ShapeDtypeStruct((S, 2 * D), _BF),
        in_specs=[any_spec] * 9,
        out_specs=any_spec,
        scratch_shapes=scratch,
        compiler_params=pltpu.CompilerParams(vmem_limit_bytes=110 * 1024 * 1024),
        name="concat_mha_rmt",
    )(A_x.reshape(S, D), A_wqkv, A_wo, B_x.reshape(S, D), B_mem0.reshape(MEM, D),
      B_Wq, B_Wk, B_Wv, B_Wo.reshape(HB * DHB, D))
    return out.reshape(1, S, 2 * D)
```
